```python
import os as _os
_os.environ.setdefault("JAX_PLATFORMS", "cpu")
import jax
import jax.numpy as jnp

def _softmax(x, axis=-1):
    return jax.nn.softmax(x, axis=axis)
def _gelu(x):
    return jax.nn.gelu(x, approximate=True)
def _silu(x):
    return jax.nn.silu(x)
def _sigmoid(x):
    return jax.nn.sigmoid(x)
def _layernorm(x, axis=-1, eps=1e-5):
    m = jnp.mean(x, axis=axis, keepdims=True)
    v = jnp.var(x, axis=axis, keepdims=True)
    return (x - m) / jnp.sqrt(v + eps)
def _scatter_add(tgt, idx, src, axis=0):
    return tgt.at[idx].add(src)
def _segment_sum(src, seg, n):
    return jax.ops.segment_sum(src, seg, n)
class _Rng:
    def __init__(self, key):
        self._k = key
    def _next(self):
        self._k, sub = jax.random.split(self._k)
        return sub
    def normal(self, shape):
        return jax.random.normal(self._next(), shape, dtype=jnp.bfloat16)
    def randint(self, lo, hi, shape):
        return jax.random.randint(self._next(), shape, lo, hi, dtype=jnp.int32)
    def uniform(self, shape, lo=0.0, hi=1.0):
        return jax.random.uniform(self._next(), shape, jnp.bfloat16, lo, hi)
    def permutation(self, n):
        return jax.random.permutation(self._next(), n)


kernel_name = 'concat_heads__mha_block__ssm_conv_s4__prompt'

def setup_inputs():
    _rng = _Rng(jax.random.key(int.from_bytes(__import__("os").urandom(4), "little")))
    _w = (lambda a: (lambda t: t.astype(jnp.bfloat16) if jnp.issubdtype(t.dtype, jnp.floating) else t)(jnp.asarray(a)))
    def _A_setup():
        B, S, D, H = 1, 2048, 448, 16
        return {
            "x": _w((lambda *s: _rng.normal(s) * 0.2)(B, S, D)),
            "wqkv": _w((lambda *s: _rng.normal(s) * 0.2)(D, 3 * D)),
            "wo": _w((lambda *s: _rng.normal(s) * 0.05)(D, D)),
        }
    _A_in = _A_setup()

    def _B_setup():
        B, L, D, N = 1, 2048, 448, 256
        A_re = -jnp.exp((lambda *s: _rng.normal(s) * 0.2)(D, N))
        A_im = jnp.pi * (lambda *s: _rng.normal(s) * 0.2)(D, N)
        B_re = (lambda *s: _rng.normal(s) * 0.2)(D, N)
        B_im = (lambda *s: _rng.normal(s) * 0.2)(D, N)
        C_re = (lambda *s: _rng.normal(s) * 0.2)(D, N)
        C_im = (lambda *s: _rng.normal(s) * 0.2)(D, N)
        log_dt = (lambda *s: _rng.normal(s) * 0.2)(D) * 0.5 - 4.0
        Dskip = (lambda *s: _rng.normal(s) * 0.05)(D)
        return {
            "u": _w((lambda *s: _rng.normal(s) * 0.05)(B, L, D)),
            "A_re": _w(A_re),
            "A_im": _w(A_im),
            "B_re": _w(B_re),
            "B_im": _w(B_im),
            "C_re": _w(C_re),
            "C_im": _w(C_im),
            "log_dt": _w(log_dt),
            "Dskip": _w(Dskip),
        }
    _B_in = _B_setup()

    return {
        "A_x": _A_in["x"],
        "A_wqkv": _A_in["wqkv"],
        "A_wo": _A_in["wo"],
        "B_u": _B_in["u"],
        "B_A_re": _B_in["A_re"],
        "B_A_im": _B_in["A_im"],
        "B_B_re": _B_in["B_re"],
        "B_B_im": _B_in["B_im"],
        "B_C_re": _B_in["C_re"],
        "B_C_im": _B_in["C_im"],
        "B_log_dt": _B_in["log_dt"],
        "B_Dskip": _B_in["Dskip"],
    }

def reference(A_x, A_wqkv, A_wo, B_u, B_A_re, B_A_im, B_B_re, B_B_im, B_C_re, B_C_im, B_log_dt, B_Dskip):
    def _A_ref(x, wqkv, wo):
        B, S, D = x.shape
        H = 16
        Dh = D // H
        qkv = (lambda x, *d: x.transpose(*d))((x @ wqkv).reshape(B, S, 3, H, Dh), 2, 0, 3, 1, 4)
        q, k, v = qkv[0], qkv[1], qkv[2]
        scores = jnp.einsum("bhqd,bhkd->bhqk", q, k) * (Dh ** -0.5)
        p = _softmax(scores, axis=-1)
        o = jnp.einsum("bhqk,bhkd->bhqd", p, v)
        return (lambda x, *d: x.transpose(*d))(o, 0, 2, 1, 3).reshape(B, S, D) @ wo

    def _B_ref(u, A_re, A_im, B_re, B_im, C_re, C_im, log_dt, Dskip):
        Bsz, L, D = u.shape
        dt = jnp.exp(log_dt)[:, None]
        A = A_re + 1j * A_im
        Bc = B_re + 1j * B_im
        Cc = C_re + 1j * C_im
        logdA = dt * A
        dB = dt * Bc
        l = (lambda x, dt: x.astype(dt))(jnp.arange(L), A_re.dtype)
        P = jnp.exp(logdA[:, :, None] * l[None, None, :])
        K = jnp.einsum("dn,dnl,dn->dl", Cc, P, dB).real
        L2 = 2 * L
        Kp = jnp.pad(K, ((0, 0), (0, L)))
        up = (lambda x, *d: x.transpose(*d))(u, 0, 2, 1)
        up = jnp.pad(up, ((0, 0), (0, 0), (0, L)))
        Kf = (lambda x, axes=(-2,-1): jnp.fft.rfft2(x.astype(jnp.float32), axes=axes))(Kp[:, None, :], axes=(-2, -1))
        Uf = (lambda x, axes=(-2,-1): jnp.fft.rfft2(x.astype(jnp.float32), axes=axes))(up[:, :, None, :], axes=(-2, -1))
        Yf = Uf * Kf[None, :, :, :]
        y = (lambda x, s, axes=(-2,-1): jnp.fft.irfft2(x, s=s, axes=axes).astype(jnp.bfloat16))(Yf, (1, L2), axes=(-2, -1))[:, :, 0, :L]
        y = (lambda x, *d: x.transpose(*d))(y, 0, 2, 1) + u * Dskip[None, None, :]
        return y

    a = _A_ref(A_x, A_wqkv, A_wo)
    b = _B_ref(B_u, B_A_re, B_A_im, B_B_re, B_B_im, B_C_re, B_C_im, B_log_dt, B_Dskip)
    return jnp.concatenate([a, b], axis=-1)
```

```python
import functools
import math

import jax
import jax.numpy as jnp
from jax import lax
import jax.experimental.pallas as pl
import jax.experimental.pallas.tpu as pltpu

F32 = jnp.float32
BF16 = jnp.bfloat16

S = 2048
D = 448
H = 16
DH = 28
HP = 32
DP = H * HP
NS = 256
DL = 2 * D
NLT = DL // 128
TQ = 256
NQ = S // TQ
CH = 128
NCH = S // CH
KROWS = 648


def _cmul(ar, ai, br, bi):
    return ar * br - ai * bi, ar * bi + ai * br


def _dot(a, b):
    return jnp.dot(a, b, preferred_element_type=F32)


def _kgen_tile(j, are_ref, aim_ref, bre_ref, bim_ref, cre_ref, cim_ref, ldt_ref,
               yr_ref, yi_ref, kd_ref):
    off = pl.multiple_of(j * 128, 128)
    sl = pl.ds(off, 128)
    dt = jnp.exp(ldt_ref[:, sl].astype(F32)).astype(BF16).astype(F32)
    lr = dt * are_ref[:, sl].astype(F32)
    li = dt * aim_ref[:, sl].astype(F32)
    dbr = dt * bre_ref[:, sl].astype(F32)
    dbi = dt * bim_ref[:, sl].astype(F32)
    cr, ci = _cmul(cre_ref[:, sl].astype(F32), cim_ref[:, sl].astype(F32), dbr, dbi)
    mag = jnp.exp(lr)
    zr = mag * jnp.cos(li)
    zi = mag * jnp.sin(li)
    pw = [(zr, zi)]
    for _ in range(11):
        r, i = pw[-1]
        pw.append((r * r - i * i, 2.0 * r * i))
    blocks = [(None, 0), (7, 0), (8, 1), (9, 2), (10, 3)]
    for blk, (l0, k) in enumerate(blocks):
        if blk != 1:
            br, bi = pw[k]
            yr = jnp.ones_like(br)
            yi = jnp.zeros_like(br)
            for b in range(16):
                yr_ref[b] = yr
                yi_ref[b] = yi
                if b < 15:
                    yr, yi = _cmul(yr, yi, br, bi)
        if l0 is None:
            xr0, xi0 = cr, ci
        else:
            xr0, xi0 = _cmul(cr, ci, pw[l0][0], pw[l0][1])
        sr, si = pw[k + 4]

        def body(a, carry, blk=blk, sr=sr, si=si):
            xr, xi = carry
            rows = []
            for b in range(16):
                t = xr * yr_ref[b] - xi * yi_ref[b]
                rows.append(jnp.sum(t, axis=0, keepdims=True))
            blockv = jnp.concatenate(rows, axis=0)
            r0 = pl.multiple_of(blk * 128 + a * 16, 16)
            kd_ref[pl.ds(r0, 16), sl] = blockv
            return _cmul(xr, xi, sr, si)

        lax.fori_loop(0, 8, body, (xr0, xi0))
    xr, _ = _cmul(cr, ci, pw[11][0], pw[11][1])
    last = jnp.sum(xr, axis=0, keepdims=True)
    row = lax.broadcasted_iota(jnp.int32, (8, 128), 0)
    kd_ref[pl.ds(640, 8), sl] = jnp.where(row == 0, last, 0.0)


def _dft_mats():
    f = lax.broadcasted_iota(jnp.int32, (CH, CH), 0)
    t = lax.broadcasted_iota(jnp.int32, (CH, CH), 1)
    ang = (((2 * f + 1) * t) % 512).astype(F32) * (2.0 * math.pi / 512.0)
    fwd = jnp.concatenate([jnp.cos(ang), -jnp.sin(ang)], axis=0)
    t2 = lax.broadcasted_iota(jnp.int32, (2 * CH, CH), 0)
    f2 = lax.broadcasted_iota(jnp.int32, (2 * CH, CH), 1)
    ang2 = (((2 * f2 + 1) * t2) % 512).astype(F32) * (2.0 * math.pi / 512.0)
    inv = jnp.concatenate([jnp.cos(ang2), -jnp.sin(ang2)], axis=1) * (2.0 / 256.0)
    return fwd, inv


def _sel_mat(chunk):
    b = lax.broadcasted_iota(jnp.int32, (CH, 136), 0)
    i = lax.broadcasted_iota(jnp.int32, (CH, 136), 1)
    l = chunk * CH + b
    if chunk < 4:
        s, sh, l0 = 2, 1, 256
    elif chunk < 8:
        s, sh, l0 = 4, 2, 512
    else:
        s, sh, l0 = 8, 3, 1024
    q = l >> sh
    rem = l & (s - 1)
    half = s // 2
    up = jnp.logical_or(rem > half, jnp.logical_and(rem == half, (q & 1) == 1))
    q = q + up.astype(jnp.int32)
    idx = q - (l0 >> sh)
    return (idx == i).astype(BF16)


def _s4_conv(u_ref, dsk_ref, kd_ref, uf_ref, kf_ref, y_ref):
    fwd, inv = _dft_mats()
    fwd_b = fwd.astype(BF16)
    inv_b = inv.astype(BF16)
    kd = kd_ref[:, 0:D] + kd_ref[:, D:2 * D]
    kdb = kd.astype(BF16)
    for a in range(NCH):
        uf_ref[a] = _dot(fwd_b, u_ref[a * CH:(a + 1) * CH, :])
        if a < 2:
            kf_ref[a] = _dot(fwd_b, kdb[a * CH:(a + 1) * CH, :])
        else:
            base = 256 if a < 4 else (384 if a < 8 else 512)
            g = _dot(fwd_b, _sel_mat(a)).astype(BF16)
            kf_ref[a] = _dot(g, kdb[base:base + 136, :])
    prev_hi = None
    for a in range(NCH):
        yr = None
        yi = None
        for a2 in range(a + 1):
            ur = uf_ref[a2, 0:CH, :]
            ui = uf_ref[a2, CH:2 * CH, :]
            kr = kf_ref[a - a2, 0:CH, :]
            ki = kf_ref[a - a2, CH:2 * CH, :]
            pr = ur * kr - ui * ki
            pi = ur * ki + ui * kr
            yr = pr if yr is None else yr + pr
            yi = pi if yi is None else yi + pi
        yf = jnp.concatenate([yr, yi], axis=0).astype(BF16)
        full = _dot(inv_b, yf)
        lo = full[0:CH, :]
        if prev_hi is not None:
            lo = lo + prev_hi
        prev_hi = full[CH:2 * CH, :]
        uu = u_ref[a * CH:(a + 1) * CH, :].astype(F32)
        ud = (uu * dsk_ref[...].astype(F32)).astype(BF16).astype(F32)
        y_ref[a * CH:(a + 1) * CH, :] = (lo.astype(BF16).astype(F32) + ud).astype(BF16)


def _kernel(x_ref, xT_ref, wq_ref, wkT_ref, wv_ref, wo_ref, u_ref,
            are_ref, aim_ref, bre_ref, bim_ref, cre_ref, cim_ref, ldt_ref, dsk_ref,
            att_ref, y_ref,
            kT_ref, v_ref, yr_ref, yi_ref, kd_ref, uf_ref, kf_ref):
    step = pl.program_id(0)

    @pl.when(step == 0)
    def _():
        kT_ref[...] = _dot(wkT_ref[...], xT_ref[...]).astype(BF16)
        v = _dot(x_ref[...], wv_ref[...])
        lane = lax.broadcasted_iota(jnp.int32, (S, DP), 1)
        v_ref[...] = jnp.where(lane % HP == DH, 1.0, v).astype(BF16)

        def kg(j, c):
            _kgen_tile(j, are_ref, aim_ref, bre_ref, bim_ref, cre_ref, cim_ref, ldt_ref,
                       yr_ref, yi_ref, kd_ref)
            return c
        lax.fori_loop(0, NLT, kg, 0)
        _s4_conv(u_ref, dsk_ref, kd_ref, uf_ref, kf_ref, y_ref)

    r0 = pl.multiple_of(step * TQ, TQ)
    xq = x_ref[pl.ds(r0, TQ), :]
    q = _dot(xq, wq_ref[...]).astype(BF16)
    scale = DH ** -0.5
    lane = lax.broadcasted_iota(jnp.int32, (TQ, 128), 1)
    o_tiles = []
    for tile in range(4):
        qt = q[:, tile * 128:(tile + 1) * 128]
        kt = kT_ref[tile * 128:(tile + 1) * 128, :]
        vt = v_ref[:, tile * 128:(tile + 1) * 128]
        ot = jnp.zeros((TQ, 128), F32)
        for hh in range(4):
            hm = (lane // HP) == hh
            qm = jnp.where(hm, qt, jnp.zeros_like(qt))
            s = _dot(qm, kt)
            m = jnp.max(s, axis=-1, keepdims=True)
            p = jnp.exp((s - m) * scale).astype(BF16)
            o = _dot(p, vt)
            l = jnp.sum(jnp.where(lane == hh * HP + DH, o, 0.0), axis=-1, keepdims=True)
            ot = jnp.where(hm, o / l, ot)
        o_tiles.append(ot.astype(BF16))
    oall = jnp.concatenate(o_tiles, axis=1)
    att_ref[...] = _dot(oall, wo_ref[...]).astype(BF16)


def _fold(p):
    return p.T.reshape(2, 128, D).transpose(1, 0, 2).reshape(128, DL)


@jax.jit
def pallas_concat_heads__mha_block__ssm_conv_s4__prompt_kernel(
    A_x: jax.Array,
    A_wqkv: jax.Array,
    A_wo: jax.Array,
    B_u: jax.Array,
    B_A_re: jax.Array,
    B_A_im: jax.Array,
    B_B_re: jax.Array,
    B_B_im: jax.Array,
    B_C_re: jax.Array,
    B_C_im: jax.Array,
    B_log_dt: jax.Array,
    B_Dskip: jax.Array,
):
    x = A_x[0]
    xT = x.T

    def padh(w):
        return jnp.pad(w.reshape(D, H, DH), ((0, 0), (0, 0), (0, HP - DH))).reshape(D, DP)

    wq = padh(A_wqkv[:, 0:D])
    wkT = padh(A_wqkv[:, D:2 * D]).T
    wv = padh(A_wqkv[:, 2 * D:3 * D])
    wo = jnp.pad(A_wo.reshape(H, DH, D), ((0, 0), (0, HP - DH), (0, 0))).reshape(DP, D)
    u = B_u[0]
    params = [_fold(p) for p in (B_A_re, B_A_im, B_B_re, B_B_im, B_C_re, B_C_im)]
    ldt = jnp.concatenate([B_log_dt, B_log_dt])[None, :]
    dsk = B_Dskip[None, :]

    def full(a):
        return pl.BlockSpec(a.shape, lambda i: (0,) * a.ndim)

    ins = [x, xT, wq, wkT, wv, wo, u] + params + [ldt, dsk]
    att, y = pl.pallas_call(
        _kernel,
        grid=(NQ,),
        in_specs=[full(a) for a in ins],
        out_specs=[pl.BlockSpec((TQ, D), lambda i: (i, 0)),
                   pl.BlockSpec((S, D), lambda i: (0, 0))],
        out_shape=[jax.ShapeDtypeStruct((S, D), BF16), jax.ShapeDtypeStruct((S, D), BF16)],
        scratch_shapes=[
            pltpu.VMEM((DP, S), BF16),
            pltpu.VMEM((S, DP), BF16),
            pltpu.VMEM((16, 128, 128), F32),
            pltpu.VMEM((16, 128, 128), F32),
            pltpu.VMEM((KROWS, DL), F32),
            pltpu.VMEM((NCH, 2 * CH, D), F32),
            pltpu.VMEM((NCH, 2 * CH, D), F32),
        ],
        compiler_params=pltpu.CompilerParams(
            dimension_semantics=("arbitrary",),
            vmem_limit_bytes=100 * 1024 * 1024,
        ),
    )(*ins)
    return jnp.concatenate([att, y], axis=-1)[None]
```

```python
import math

import jax
import jax.numpy as jnp
from jax import lax
import jax.experimental.pallas as pl
import jax.experimental.pallas.tpu as pltpu

F32 = jnp.float32
BF16 = jnp.bfloat16

S = 2048
D = 448
H = 16
DH = 28
HP = 32
DP = H * HP
DL = 2 * D
DPAD = 512
NLT = DL // 128
TQ = 256
NQ = S // TQ
NIT = NQ * H
CH = 128
NCH = S // CH
KROWS = 656
UNROLL = 4
HU_PER_IT = 5


def _cmul(ar, ai, br, bi):
    return ar * br - ai * bi, ar * bi + ai * br


def _dot(a, b):
    return jnp.dot(a, b, preferred_element_type=F32)


SR = 16


def _kgen_setup_rows(j, c, prm_ref, dt_ref, xr_ref, xi_ref, yr_ref, yi_ref, k2_ref):
    sl = pl.ds(pl.multiple_of(j * 128, 128), 128)
    rs = pl.ds(pl.multiple_of(c * SR, SR), SR)
    dt = dt_ref[:, sl]
    lr = dt * prm_ref[0, rs, sl]
    li = dt * prm_ref[1, rs, sl]
    dbr = dt * prm_ref[2, rs, sl]
    dbi = dt * prm_ref[3, rs, sl]
    cr, ci = _cmul(prm_ref[4, rs, sl], prm_ref[5, rs, sl], dbr, dbi)
    mag = jnp.exp(lr)
    zr = mag * jnp.cos(li)
    zi = mag * jnp.sin(li)
    pw = [(zr, zi)]
    for _ in range(11):
        r, i = pw[-1]
        pw.append((r * r - i * i, 2.0 * r * i))
    xr, _ = _cmul(cr, ci, pw[11][0], pw[11][1])
    k2_ref[rs, sl] = xr
    for k in range(4):
        yr, yi = jnp.ones_like(zr), jnp.zeros_like(zr)
        for b in range(16):
            yr_ref[k * 16 + b, rs, :] = yr
            yi_ref[k * 16 + b, rs, :] = yi
            if b < 15:
                yr, yi = _cmul(yr, yi, pw[k][0], pw[k][1])
    blocks = [(None, 0), (7, 0), (8, 1), (9, 2), (10, 3)]
    for blk, (l0, k) in enumerate(blocks):
        if l0 is None:
            xr, xi = (cr, ci)
        else:
            xr, xi = _cmul(cr, ci, pw[l0][0], pw[l0][1])
        sr, si = pw[k + 4]
        for a in range(8):
            xr_ref[blk * 8 + a, rs, :] = xr
            xi_ref[blk * 8 + a, rs, :] = xi
            if a < 7:
                xr, xi = _cmul(xr, xi, sr, si)


def _kgen_unit(j, uu, xr_ref, xi_ref, yr_ref, yi_ref, kd_ref):
    off = pl.multiple_of(j * 128, 128)
    blk = uu >> 3
    xa = (uu >> 1) * 2
    bh = uu & 1
    ybase = jnp.maximum(blk - 1, 0) * 16 + bh * 8
    acc0 = [None] * 8
    acc1 = [None] * 8
    for r in range(16):
        rs = slice(r * 8, (r + 1) * 8)
        xr0 = xr_ref[xa, rs, :]
        xi0 = xi_ref[xa, rs, :]
        xr1 = xr_ref[xa + 1, rs, :]
        xi1 = xi_ref[xa + 1, rs, :]
        for b in range(8):
            yr = yr_ref[ybase + b, rs, :]
            yi = yi_ref[ybase + b, rs, :]
            t0 = xr0 * yr - xi0 * yi
            t1 = xr1 * yr - xi1 * yi
            acc0[b] = t0 if acc0[b] is None else acc0[b] + t0
            acc1[b] = t1 if acc1[b] is None else acc1[b] + t1
    b0 = jnp.concatenate([jnp.sum(a, axis=0, keepdims=True) for a in acc0], axis=0)
    b1 = jnp.concatenate([jnp.sum(a, axis=0, keepdims=True) for a in acc1], axis=0)
    r0 = pl.multiple_of(xa * 16 + bh * 8, 8)
    kd_ref[pl.ds(r0, 8), pl.ds(off, 128)] = b0
    kd_ref[pl.ds(r0 + 16, 8), pl.ds(off, 128)] = b1


def _dft_mats():
    f = lax.broadcasted_iota(jnp.int32, (CH, CH), 0)
    t = lax.broadcasted_iota(jnp.int32, (CH, CH), 1)
    ang = (((2 * f + 1) * t) % 512).astype(F32) * (2.0 * math.pi / 512.0)
    fwd = jnp.concatenate([jnp.cos(ang), -jnp.sin(ang)], axis=0)
    t2 = lax.broadcasted_iota(jnp.int32, (2 * CH, CH), 0)
    f2 = lax.broadcasted_iota(jnp.int32, (2 * CH, CH), 1)
    ang2 = (((2 * f2 + 1) * t2) % 512).astype(F32) * (2.0 * math.pi / 512.0)
    inv = jnp.concatenate([jnp.cos(ang2), -jnp.sin(ang2)], axis=1) * (2.0 / 256.0)
    return fwd, inv


def _sel_mat(s, sh, width):
    b = lax.broadcasted_iota(jnp.int32, (CH, width), 0)
    i = lax.broadcasted_iota(jnp.int32, (CH, width), 1)
    q = b >> sh
    rem = b & (s - 1)
    half = s // 2
    up = jnp.logical_or(rem > half, jnp.logical_and(rem == half, (q & 1) == 1))
    q = q + up.astype(jnp.int32)
    return (q == i).astype(BF16)


def _s4_conv(uT_ref, dsk_ref, kd_ref, k2_ref, uf_ref, kf_ref, out_ref, out_hbm, out_sems, fwd_ref, inv_ref, kdb_ref,
             yf_ref, hi_ref, uc_ref, g_ref):
    fwd, inv = _dft_mats()
    fwd_ref[...] = fwd.astype(BF16)
    inv_ref[...] = inv.astype(BF16)
    last = jnp.sum(k2_ref[...], axis=0, keepdims=True)
    row = lax.broadcasted_iota(jnp.int32, (16, DL), 0)
    kd_ref[pl.ds(640, 16), :] = jnp.where(row == 0, last, 0.0)
    kdb_ref[...] = (kd_ref[:, 0:D] + kd_ref[:, D:2 * D]).astype(BF16)
    zpad = jnp.zeros((2 * CH, DPAD - D), F32)

    def fwd_u(a, c):
        r0 = pl.multiple_of(a * CH, CH)
        uc = uT_ref[:, pl.ds(r0, CH)].astype(F32).T
        uc_ref[pl.ds(r0, CH), :] = uc
        uf_ref[a, :, 0:D] = _dot(fwd_ref[...], uc.astype(BF16))
        uf_ref[a, :, D:DPAD] = zpad
        kf_ref[a, :, D:DPAD] = zpad
        return c
    lax.fori_loop(0, NCH, fwd_u, 0)

    def fwd_k0(a, c):
        r0 = pl.multiple_of(a * CH, CH)
        kf_ref[a, :, 0:D] = _dot(fwd_ref[...], kdb_ref[pl.ds(r0, CH), :])
        return c
    lax.fori_loop(0, 2, fwd_k0, 0)

    for (c0, c1, s, sh, base) in ((2, 4, 2, 1, 256), (4, 8, 4, 2, 384), (8, 16, 8, 3, 512)):
        width = CH // s + 16
        g_ref[:, 0:width] = _dot(fwd_ref[...], _sel_mat(s, sh, width)).astype(BF16)

        def fwd_k(a, c, c0=c0, s=s, base=base, width=width):
            r0 = pl.multiple_of(base + (a - c0) * (CH // s), 16)
            kf_ref[a, :, 0:D] = _dot(g_ref[:, 0:width], kdb_ref[pl.ds(r0, width), :])
            return c
        lax.fori_loop(c0, c1, fwd_k, 0)

    RB = 32
    NRB = CH // RB

    def blk_conv(i, c):
        rb = i & (NRB - 1)
        lt = i >> 2
        rr = pl.ds(pl.multiple_of(rb * RB, RB), RB)
        ri = pl.ds(pl.multiple_of(CH + rb * RB, RB), RB)
        ll = pl.ds(pl.multiple_of(lt * 128, 128), 128)
        for a in range(NCH):
            accr = None
            acci = None
            for a2 in range(a + 1):
                ur = uf_ref[a2, rr, ll]
                ui = uf_ref[a2, ri, ll]
                kr = kf_ref[a - a2, rr, ll]
                ki = kf_ref[a - a2, ri, ll]
                pr = ur * kr - ui * ki
                pi = ur * ki + ui * kr
                accr = pr if accr is None else accr + pr
                acci = pi if acci is None else acci + pi
            yf_ref[a, rr, ll] = accr.astype(BF16)
            yf_ref[a, ri, ll] = acci.astype(BF16)
        return c
    lax.fori_loop(0, NRB * (DPAD // 128), blk_conv, 0)

    hi_ref[...] = jnp.zeros(hi_ref.shape, F32)

    def out_chunk(a, c):
        full = _dot(inv_ref[...], yf_ref[a, :, 0:D])
        lo = full[0:CH, :] + hi_ref[...]
        hi_ref[...] = full[CH:2 * CH, :]
        r0 = pl.multiple_of(a * CH, CH)
        uu = uc_ref[pl.ds(r0, CH), :]
        ud = (uu * dsk_ref[...].astype(F32)).astype(BF16).astype(F32)
        out_ref[pl.ds(r0, CH), D:2 * D] = (lo.astype(BF16).astype(F32) + ud).astype(BF16)
        pltpu.make_async_copy(out_ref.at[pl.ds(r0, CH), :], out_hbm.at[0, pl.ds(r0, CH), :],
                              out_sems.at[a]).start()
        return c
    lax.fori_loop(0, NCH, out_chunk, 0)
    for a in range(NCH):
        pltpu.make_async_copy(out_ref.at[pl.ds(a * CH, CH), :],
                              out_hbm.at[0, pl.ds(a * CH, CH), :], out_sems.at[a]).wait()


def _kernel(xT_hbm, wqkv_hbm, wo_ref, uT_hbm, are_ref, aim_ref, bre_ref, bim_ref, cre_ref, cim_ref,
            ldt_ref, dsk_ref,
            out_hbm,
            xT_ref, wqkv_ref, uT_ref, out_ref, in_sems, out_sems,
            q_ref, kT_ref, v_ref, o_ref, sa_ref, sb_ref, sc_ref, sd_ref,
            wpT_ref, wop_ref, prm_ref, dt_ref,
            xr_ref, xi_ref, yr_ref, yi_ref, kd_ref, k2_ref, uf_ref, kf_ref,
            fwd_ref, inv_ref, kdb_ref, yf_ref, hi_ref, uc_ref, g_ref):
    lane = lax.broadcasted_iota(jnp.int32, (TQ, 128), 1)
    lane_head = lane // HP
    qscale = (DH ** -0.5) * math.log2(math.e)

    cp_w = pltpu.make_async_copy(wqkv_hbm, wqkv_ref, in_sems.at[0])
    cp_x = pltpu.make_async_copy(xT_hbm, xT_ref, in_sems.at[1])
    cp_u = pltpu.make_async_copy(uT_hbm, uT_ref, in_sems.at[2])
    cp_w.start()
    cp_x.start()
    cp_u.start()

    for i, p_ref in enumerate((are_ref, aim_ref, bre_ref, bim_ref, cre_ref, cim_ref)):
        pt = p_ref[...].astype(F32).T
        prm_ref[i, :, 0:D] = pt[0:128, :]
        prm_ref[i, :, D:DL] = pt[128:256, :]
    dt = jnp.exp(ldt_ref[...].astype(F32)).astype(BF16).astype(F32)
    dt_ref[:, 0:D] = dt
    dt_ref[:, D:DL] = dt

    def kgen_tile(j, carry):
        def setup(c, cc):
            _kgen_setup_rows(j, c, prm_ref, dt_ref, xr_ref, xi_ref, yr_ref, yi_ref, k2_ref)
            return cc
        lax.fori_loop(0, 128 // SR, setup, 0)

        def unit(uu, cc):
            _kgen_unit(j, uu, xr_ref, xi_ref, yr_ref, yi_ref, kd_ref)
            return cc
        lax.fori_loop(0, 40, unit, 0)
        return carry
    lax.fori_loop(0, NLT, kgen_tile, 0)

    cp_w.wait()
    cp_x.wait()

    wT = wqkv_ref[...].astype(F32).T.astype(BF16)
    zrows = jnp.zeros((HP - DH, D), BF16)
    for g in range(3 * H):
        wpT_ref[g * HP:g * HP + DH, :] = wT[g * DH:(g + 1) * DH, :]
        wpT_ref[g * HP + DH:(g + 1) * HP, :] = zrows
    for g in range(H):
        wop_ref[g * HP:g * HP + DH, :] = wo_ref[g * DH:(g + 1) * DH, :]
        wop_ref[g * HP + DH:(g + 1) * HP, :] = zrows

    def proj(i, c):
        r0 = pl.multiple_of(i * TQ, TQ)
        xb = xT_ref[:, pl.ds(r0, TQ)]
        qkvT = _dot(wpT_ref[...], xb)
        q = (qkvT[0:DP, :] * qscale).T.astype(BF16)
        kt = qkvT[DP:2 * DP, :].astype(BF16)
        rowh = lax.broadcasted_iota(jnp.int32, (DP, TQ), 0)
        v = jnp.where(rowh % HP == DH, 1.0, qkvT[2 * DP:3 * DP, :]).T.astype(BF16)
        for t in range(4):
            q_ref[t, pl.ds(r0, TQ), :] = q[:, t * 128:(t + 1) * 128]
            v_ref[t, pl.ds(r0, TQ), :] = v[:, t * 128:(t + 1) * 128]
            kT_ref[t, :, pl.ds(r0, TQ)] = kt[t * 128:(t + 1) * 128, :]
            o_ref[t, pl.ds(r0, TQ), :] = jnp.zeros((TQ, 128), BF16)
        return c
    lax.fori_loop(0, NQ, proj, 0)

    def scores(it):
        qb = it >> 4
        h = it & 15
        t = h >> 2
        r0 = pl.multiple_of(qb * TQ, TQ)
        qt = q_ref[t, pl.ds(r0, TQ), :]
        qm = jnp.where(lane_head == (h & 3), qt, jnp.zeros_like(qt))
        return _dot(qm, kT_ref[t])

    def softmax_pv(it, s_in_ref, dep):
        qb = it >> 4
        h = it & 15
        t = h >> 2
        hh = h & 3
        r0 = pl.multiple_of(qb * TQ, TQ)
        s = s_in_ref[...]
        m = jnp.max(s, axis=-1, keepdims=True)
        if dep is not None:
            m = jnp.maximum(m, dep)
        p = jnp.exp2(s - m).astype(BF16)
        o = _dot(p, v_ref[t])
        l = jnp.sum(jnp.where(lane == hh * HP + DH, o, 0.0), axis=-1, keepdims=True)
        on = (o / l).astype(BF16)
        o_ref[t, pl.ds(r0, TQ), :] = jnp.where(lane_head == hh, on, o_ref[t, pl.ds(r0, TQ), :])

    sbufs = (sa_ref, sb_ref, sc_ref, sd_ref)
    sa_ref[...] = scores(0)
    sb_ref[...] = scores(1)

    def main(i4, c):
        it0 = i4 * UNROLL
        j = jnp.minimum(it0 >> 4, NLT - 1)
        jn = jnp.minimum(j + 1, NLT - 1)
        parn = (j + 1) & 1
        for k4 in range(UNROLL):
            it = it0 + k4
            sbufs[(k4 + 2) % 4][...] = scores(jnp.minimum(it + 2, NIT - 1))
            softmax_pv(it, sbufs[k4 % 4], None)
        return c
    lax.fori_loop(0, NIT // UNROLL, main, 0)

    def oproj(i, c):
        r0 = pl.multiple_of(i * TQ, TQ)
        oall = jnp.concatenate([o_ref[t, pl.ds(r0, TQ), :] for t in range(4)], axis=1)
        out_ref[pl.ds(r0, TQ), 0:D] = _dot(oall, wop_ref[...]).astype(BF16)
        return c
    lax.fori_loop(0, NQ, oproj, 0)

    cp_u.wait()
    _s4_conv(uT_ref, dsk_ref, kd_ref, k2_ref, uf_ref, kf_ref, out_ref, out_hbm, out_sems, fwd_ref, inv_ref, kdb_ref,
             yf_ref, hi_ref, uc_ref, g_ref)


@jax.jit
def pallas_concat_heads__mha_block__ssm_conv_s4__prompt_kernel(
    A_x: jax.Array,
    A_wqkv: jax.Array,
    A_wo: jax.Array,
    B_u: jax.Array,
    B_A_re: jax.Array,
    B_A_im: jax.Array,
    B_B_re: jax.Array,
    B_B_im: jax.Array,
    B_C_re: jax.Array,
    B_C_im: jax.Array,
    B_log_dt: jax.Array,
    B_Dskip: jax.Array,
):
    ins = [A_x[0].T, A_wqkv, A_wo, B_u[0].T, B_A_re, B_A_im, B_B_re, B_B_im, B_C_re, B_C_im,
           B_log_dt.reshape(1, D), B_Dskip.reshape(1, D)]
    any_spec = pl.BlockSpec(memory_space=pl.ANY)
    vmem_spec = pl.BlockSpec(memory_space=pltpu.VMEM)
    out = pl.pallas_call(
        _kernel,
        in_specs=[any_spec, any_spec, vmem_spec, any_spec] + [vmem_spec] * 8,
        out_specs=any_spec,
        out_shape=jax.ShapeDtypeStruct((1, S, 2 * D), BF16),
        scratch_shapes=[
            pltpu.VMEM((D, S), BF16),
            pltpu.VMEM((D, 3 * D), BF16),
            pltpu.VMEM((D, S), BF16),
            pltpu.VMEM((S, 2 * D), BF16),
            pltpu.SemaphoreType.DMA((3,)),
            pltpu.SemaphoreType.DMA((NCH,)),
            pltpu.VMEM((4, S, 128), BF16),
            pltpu.VMEM((4, 128, S), BF16),
            pltpu.VMEM((4, S, 128), BF16),
            pltpu.VMEM((4, S, 128), BF16),
            pltpu.VMEM((TQ, S), F32),
            pltpu.VMEM((TQ, S), F32),
            pltpu.VMEM((TQ, S), F32),
            pltpu.VMEM((TQ, S), F32),
            pltpu.VMEM((3 * DP, D), BF16),
            pltpu.VMEM((DP, D), BF16),
            pltpu.VMEM((6, 128, DL), F32),
            pltpu.VMEM((1, DL), F32),
            pltpu.VMEM((40, 128, 128), F32),
            pltpu.VMEM((40, 128, 128), F32),
            pltpu.VMEM((64, 128, 128), F32),
            pltpu.VMEM((64, 128, 128), F32),
            pltpu.VMEM((KROWS, DL), F32),
            pltpu.VMEM((128, DL), F32),
            pltpu.VMEM((NCH, 2 * CH, DPAD), F32),
            pltpu.VMEM((NCH, 2 * CH, DPAD), F32),
            pltpu.VMEM((2 * CH, CH), BF16),
            pltpu.VMEM((2 * CH, 2 * CH), BF16),
            pltpu.VMEM((KROWS, D), BF16),
            pltpu.VMEM((NCH, 2 * CH, DPAD), BF16),
            pltpu.VMEM((CH, D), F32),
            pltpu.VMEM((S, D), F32),
            pltpu.VMEM((2 * CH, 128), BF16),
        ],
        compiler_params=pltpu.CompilerParams(
            vmem_limit_bytes=100 * 1024 * 1024,
        ),
    )(*ins)
    return out
```

```python
import math

import jax
import jax.numpy as jnp
from jax import lax
import jax.experimental.pallas as pl
import jax.experimental.pallas.tpu as pltpu

F32 = jnp.float32
BF16 = jnp.bfloat16

S = 2048
D = 448
H = 16
DH = 28
HP = 32
DP = H * HP
DL = 2 * D
DPAD = 512
NLT = DL // 128
TQ = 512
NQ = S // TQ
NIT = NQ * H
CH = 128
NCH = S // CH
KROWS = 656
UNROLL = 4
HU_PER_IT = 5


def _cmul(ar, ai, br, bi):
    return ar * br - ai * bi, ar * bi + ai * br


def _dot(a, b):
    return jnp.dot(a, b, preferred_element_type=F32)


SR = 16


def _kgen_setup_rows(j, c, prm_ref, dt_ref, xr_ref, xi_ref, yr_ref, yi_ref, k2_ref):
    sl = pl.ds(pl.multiple_of(j * 128, 128), 128)
    rs = pl.ds(pl.multiple_of(c * SR, SR), SR)
    dt = dt_ref[:, sl]
    lr = dt * prm_ref[0, rs, sl]
    li = dt * prm_ref[1, rs, sl]
    dbr = dt * prm_ref[2, rs, sl]
    dbi = dt * prm_ref[3, rs, sl]
    cr, ci = _cmul(prm_ref[4, rs, sl], prm_ref[5, rs, sl], dbr, dbi)
    mag = jnp.exp(lr)
    zr = mag * jnp.cos(li)
    zi = mag * jnp.sin(li)
    pw = [(zr, zi)]
    for _ in range(11):
        r, i = pw[-1]
        pw.append((r * r - i * i, 2.0 * r * i))
    xr, _ = _cmul(cr, ci, pw[11][0], pw[11][1])
    k2_ref[rs, sl] = xr
    yr, yi = jnp.ones_like(zr), jnp.zeros_like(zr)
    for e in range(16):
        yr_ref[e, rs, :] = yr
        yi_ref[e, rs, :] = yi
        if e < 15:
            yr, yi = _cmul(yr, yi, zr, zi)
    for k in range(1, 4):
        yr, yi = pw[k + 3]
        for b in range(8):
            yr_ref[8 + k * 8 + b, rs, :] = yr
            yi_ref[8 + k * 8 + b, rs, :] = yi
            if b < 7:
                yr, yi = _cmul(yr, yi, pw[k][0], pw[k][1])
    blocks = [(None, 0), (7, 0), (8, 1), (9, 2), (10, 3)]
    for blk, (l0, k) in enumerate(blocks):
        if l0 is None:
            xr, xi = (cr, ci)
        else:
            xr, xi = _cmul(cr, ci, pw[l0][0], pw[l0][1])
        sr, si = pw[k + 4]
        for a in range(8):
            xr_ref[blk * 8 + a, rs, :] = xr
            xi_ref[blk * 8 + a, rs, :] = xi
            if a < 7:
                xr, xi = _cmul(xr, xi, sr, si)


def _pow_id(e):
    if e < 16:
        return e
    if e < 32:
        return 8 + (e >> 1)
    if e < 64:
        return 16 + (e >> 2)
    return 24 + (e >> 3)


def _kgen_unit(j, blk, ap, bh, xr_ref, xi_ref, yr_ref, yi_ref, kd_ref):
    off = pl.multiple_of(j * 128, 128)
    xa = blk * 8 + 2 * ap
    yid = [_pow_id((bh * 8 + b) << max(blk - 1, 0)) for b in range(8)]
    acc0 = [None] * 8
    acc1 = [None] * 8
    for r in range(16):
        rs = slice(r * 8, (r + 1) * 8)
        xr0 = xr_ref[xa, rs, :]
        xi0 = xi_ref[xa, rs, :]
        xr1 = xr_ref[xa + 1, rs, :]
        xi1 = xi_ref[xa + 1, rs, :]
        for b in range(8):
            yr = yr_ref[yid[b], rs, :]
            yi = yi_ref[yid[b], rs, :]
            t0 = xr0 * yr - xi0 * yi
            t1 = xr1 * yr - xi1 * yi
            acc0[b] = t0 if acc0[b] is None else acc0[b] + t0
            acc1[b] = t1 if acc1[b] is None else acc1[b] + t1
    b0 = jnp.concatenate([jnp.sum(a, axis=0, keepdims=True) for a in acc0], axis=0)
    b1 = jnp.concatenate([jnp.sum(a, axis=0, keepdims=True) for a in acc1], axis=0)
    r0 = pl.multiple_of(xa * 16 + bh * 8, 8)
    kd_ref[pl.ds(r0, 8), pl.ds(off, 128)] = b0
    kd_ref[pl.ds(r0 + 16, 8), pl.ds(off, 128)] = b1


def _dft_mats():
    f = lax.broadcasted_iota(jnp.int32, (CH, CH), 0)
    t = lax.broadcasted_iota(jnp.int32, (CH, CH), 1)
    ang = (((2 * f + 1) * t) % 512).astype(F32) * (2.0 * math.pi / 512.0)
    fwd = jnp.concatenate([jnp.cos(ang), -jnp.sin(ang)], axis=0)
    t2 = lax.broadcasted_iota(jnp.int32, (2 * CH, CH), 0)
    f2 = lax.broadcasted_iota(jnp.int32, (2 * CH, CH), 1)
    ang2 = (((2 * f2 + 1) * t2) % 512).astype(F32) * (2.0 * math.pi / 512.0)
    inv = jnp.concatenate([jnp.cos(ang2), -jnp.sin(ang2)], axis=1) * (2.0 / 256.0)
    return fwd, inv


def _sel_mat(s, sh, width):
    b = lax.broadcasted_iota(jnp.int32, (CH, width), 0)
    i = lax.broadcasted_iota(jnp.int32, (CH, width), 1)
    q = b >> sh
    rem = b & (s - 1)
    half = s // 2
    up = jnp.logical_or(rem > half, jnp.logical_and(rem == half, (q & 1) == 1))
    q = q + up.astype(jnp.int32)
    return (q == i).astype(BF16)


def _s4_conv(uT_ref, dsk_ref, kd_ref, k2_ref, uf_ref, kf_ref, out_ref, out_hbm, out_sems, fwd_ref, inv_ref, kdb_ref,
             yf_ref, hi_ref, uc_ref, g_ref):
    fwd, inv = _dft_mats()
    fwd_ref[...] = fwd.astype(BF16)
    inv_ref[...] = inv.astype(BF16)
    last = jnp.sum(k2_ref[...], axis=0, keepdims=True)
    row = lax.broadcasted_iota(jnp.int32, (16, DL), 0)
    kd_ref[pl.ds(640, 16), :] = jnp.where(row == 0, last, 0.0)
    kdb_ref[...] = (kd_ref[:, 0:D] + kd_ref[:, D:2 * D]).astype(BF16)
    zpad = jnp.zeros((2 * CH, DPAD - D), F32)

    def fwd_u(a, c):
        r0 = pl.multiple_of(a * CH, CH)
        uc = uT_ref[:, pl.ds(r0, CH)].astype(F32).T
        uc_ref[pl.ds(r0, CH), :] = uc
        uf_ref[a, :, 0:D] = _dot(fwd_ref[...], uc.astype(BF16))
        uf_ref[a, :, D:DPAD] = zpad
        kf_ref[a, :, D:DPAD] = zpad
        return c
    lax.fori_loop(0, NCH, fwd_u, 0)

    def fwd_k0(a, c):
        r0 = pl.multiple_of(a * CH, CH)
        kf_ref[a, :, 0:D] = _dot(fwd_ref[...], kdb_ref[pl.ds(r0, CH), :])
        return c
    lax.fori_loop(0, 2, fwd_k0, 0)

    for (c0, c1, s, sh, base) in ((2, 4, 2, 1, 256), (4, 8, 4, 2, 384), (8, 16, 8, 3, 512)):
        width = CH // s + 16
        g_ref[:, 0:width] = _dot(fwd_ref[...], _sel_mat(s, sh, width)).astype(BF16)

        def fwd_k(a, c, c0=c0, s=s, base=base, width=width):
            r0 = pl.multiple_of(base + (a - c0) * (CH // s), 16)
            kf_ref[a, :, 0:D] = _dot(g_ref[:, 0:width], kdb_ref[pl.ds(r0, width), :])
            return c
        lax.fori_loop(c0, c1, fwd_k, 0)

    RB = 8
    NRB = CH // RB

    def blk_conv(i, c):
        rb = i & (NRB - 1)
        lt = i >> 4
        rr = pl.ds(pl.multiple_of(rb * RB, RB), RB)
        ri = pl.ds(pl.multiple_of(CH + rb * RB, RB), RB)
        ll = pl.ds(pl.multiple_of(lt * 128, 128), 128)
        for a in range(NCH):
            accr = None
            acci = None
            for a2 in range(a + 1):
                ur = uf_ref[a2, rr, ll]
                ui = uf_ref[a2, ri, ll]
                kr = kf_ref[a - a2, rr, ll]
                ki = kf_ref[a - a2, ri, ll]
                pr = ur * kr - ui * ki
                pi = ur * ki + ui * kr
                accr = pr if accr is None else accr + pr
                acci = pi if acci is None else acci + pi
            yf_ref[a, rr, ll] = accr.astype(BF16)
            yf_ref[a, ri, ll] = acci.astype(BF16)
        return c
    lax.fori_loop(0, NRB * (DPAD // 128), blk_conv, 0)

    hi_ref[...] = jnp.zeros(hi_ref.shape, F32)

    def out_chunk(a, c):
        full = _dot(inv_ref[...], yf_ref[a, :, 0:D])
        lo = full[0:CH, :] + hi_ref[...]
        hi_ref[...] = full[CH:2 * CH, :]
        r0 = pl.multiple_of(a * CH, CH)
        uu = uc_ref[pl.ds(r0, CH), :]
        ud = (uu * dsk_ref[...].astype(F32)).astype(BF16).astype(F32)
        out_ref[pl.ds(r0, CH), D:2 * D] = (lo.astype(BF16).astype(F32) + ud).astype(BF16)
        pltpu.make_async_copy(out_ref.at[pl.ds(r0, CH), :], out_hbm.at[0, pl.ds(r0, CH), :],
                              out_sems.at[a]).start()
        return c
    lax.fori_loop(0, NCH, out_chunk, 0)
    for a in range(NCH):
        pltpu.make_async_copy(out_ref.at[pl.ds(a * CH, CH), :],
                              out_hbm.at[0, pl.ds(a * CH, CH), :], out_sems.at[a]).wait()


def _kernel(xT_hbm, wqkv_hbm, wo_ref, uT_hbm, are_ref, aim_ref, bre_ref, bim_ref, cre_ref, cim_ref,
            ldt_ref, dsk_ref,
            out_hbm,
            xT_ref, wqkv_ref, uT_ref, out_ref, in_sems, out_sems,
            q_ref, kT_ref, v_ref, o_ref, sa_ref, sb_ref, sc_ref, sd_ref,
            wpT_ref, wop_ref, prm_ref, dt_ref,
            xr_ref, xi_ref, yr_ref, yi_ref, kd_ref, k2_ref, uf_ref, kf_ref,
            fwd_ref, inv_ref, kdb_ref, yf_ref, hi_ref, uc_ref, g_ref):
    lane = lax.broadcasted_iota(jnp.int32, (TQ, 128), 1)
    lane_head = lane // HP
    qscale = (DH ** -0.5) * math.log2(math.e)

    cp_w = pltpu.make_async_copy(wqkv_hbm, wqkv_ref, in_sems.at[0])
    cp_x = pltpu.make_async_copy(xT_hbm, xT_ref, in_sems.at[1])
    cp_u = pltpu.make_async_copy(uT_hbm, uT_ref, in_sems.at[2])
    cp_w.start()
    cp_x.start()
    cp_u.start()

    for i, p_ref in enumerate((are_ref, aim_ref, bre_ref, bim_ref, cre_ref, cim_ref)):
        pt = p_ref[...].astype(F32).T
        prm_ref[i, :, 0:D] = pt[0:128, :]
        prm_ref[i, :, D:DL] = pt[128:256, :]
    dt = jnp.exp(ldt_ref[...].astype(F32)).astype(BF16).astype(F32)
    dt_ref[:, 0:D] = dt
    dt_ref[:, D:DL] = dt

    def kgen_tile(j, carry):
        def setup(c, cc):
            _kgen_setup_rows(j, c, prm_ref, dt_ref, xr_ref, xi_ref, yr_ref, yi_ref, k2_ref)
            return cc
        lax.fori_loop(0, 128 // SR, setup, 0)

        for blk in range(5):
            for bh in range(2):
                def unit(ap, cc, blk=blk, bh=bh):
                    _kgen_unit(j, blk, ap, bh, xr_ref, xi_ref, yr_ref, yi_ref, kd_ref)
                    return cc
                lax.fori_loop(0, 4, unit, 0)
        return carry
    lax.fori_loop(0, NLT, kgen_tile, 0)

    cp_w.wait()
    cp_x.wait()

    wT = wqkv_ref[...].astype(F32).T.astype(BF16)
    zrows = jnp.zeros((HP - DH, D), BF16)
    for g in range(3 * H):
        wpT_ref[g * HP:g * HP + DH, :] = wT[g * DH:(g + 1) * DH, :]
        wpT_ref[g * HP + DH:(g + 1) * HP, :] = zrows
    for g in range(H):
        wop_ref[g * HP:g * HP + DH, :] = wo_ref[g * DH:(g + 1) * DH, :]
        wop_ref[g * HP + DH:(g + 1) * HP, :] = zrows

    def proj(i, c):
        r0 = pl.multiple_of(i * TQ, TQ)
        xb = xT_ref[:, pl.ds(r0, TQ)]
        qkvT = _dot(wpT_ref[...], xb)
        q = (qkvT[0:DP, :] * qscale).T.astype(BF16)
        kt = qkvT[DP:2 * DP, :].astype(BF16)
        rowh = lax.broadcasted_iota(jnp.int32, (DP, TQ), 0)
        v = jnp.where(rowh % HP == DH, 1.0, qkvT[2 * DP:3 * DP, :]).T.astype(BF16)
        for t in range(4):
            q_ref[t, pl.ds(r0, TQ), :] = q[:, t * 128:(t + 1) * 128]
            v_ref[t, pl.ds(r0, TQ), :] = v[:, t * 128:(t + 1) * 128]
            kT_ref[t, :, pl.ds(r0, TQ)] = kt[t * 128:(t + 1) * 128, :]
            o_ref[t, pl.ds(r0, TQ), :] = jnp.zeros((TQ, 128), BF16)
        return c
    lax.fori_loop(0, NQ, proj, 0)

    def scores(it):
        qb = it >> 4
        h = it & 15
        t = h >> 2
        r0 = pl.multiple_of(qb * TQ, TQ)
        qt = q_ref[t, pl.ds(r0, TQ), :]
        qm = jnp.where(lane_head == (h & 3), qt, jnp.zeros_like(qt))
        return _dot(qm, kT_ref[t])

    def softmax_pv(it, s_in_ref, dep):
        qb = it >> 4
        h = it & 15
        t = h >> 2
        hh = h & 3
        r0 = pl.multiple_of(qb * TQ, TQ)
        s = s_in_ref[...]
        m = jnp.max(s, axis=-1, keepdims=True)
        if dep is not None:
            m = jnp.maximum(m, dep)
        p = jnp.exp2(s - m).astype(BF16)
        o = _dot(p, v_ref[t])
        l = jnp.sum(jnp.where(lane == hh * HP + DH, o, 0.0), axis=-1, keepdims=True)
        on = (o / l).astype(BF16)
        o_ref[t, pl.ds(r0, TQ), :] = jnp.where(lane_head == hh, on, o_ref[t, pl.ds(r0, TQ), :])

    sbufs = (sa_ref, sb_ref, sc_ref, sd_ref)
    sa_ref[...] = scores(0)
    sb_ref[...] = scores(1)

    def main(i4, c):
        it0 = i4 * UNROLL
        j = jnp.minimum(it0 >> 4, NLT - 1)
        jn = jnp.minimum(j + 1, NLT - 1)
        parn = (j + 1) & 1
        for k4 in range(UNROLL):
            it = it0 + k4
            sbufs[(k4 + 2) % 4][...] = scores(jnp.minimum(it + 2, NIT - 1))
            softmax_pv(it, sbufs[k4 % 4], None)
        return c
    lax.fori_loop(0, NIT // UNROLL, main, 0)

    def oproj(i, c):
        r0 = pl.multiple_of(i * TQ, TQ)
        oall = jnp.concatenate([o_ref[t, pl.ds(r0, TQ), :] for t in range(4)], axis=1)
        out_ref[pl.ds(r0, TQ), 0:D] = _dot(oall, wop_ref[...]).astype(BF16)
        return c
    lax.fori_loop(0, NQ, oproj, 0)

    cp_u.wait()
    _s4_conv(uT_ref, dsk_ref, kd_ref, k2_ref, uf_ref, kf_ref, out_ref, out_hbm, out_sems, fwd_ref, inv_ref, kdb_ref,
             yf_ref, hi_ref, uc_ref, g_ref)


@jax.jit
def pallas_concat_heads__mha_block__ssm_conv_s4__prompt_kernel(
    A_x: jax.Array,
    A_wqkv: jax.Array,
    A_wo: jax.Array,
    B_u: jax.Array,
    B_A_re: jax.Array,
    B_A_im: jax.Array,
    B_B_re: jax.Array,
    B_B_im: jax.Array,
    B_C_re: jax.Array,
    B_C_im: jax.Array,
    B_log_dt: jax.Array,
    B_Dskip: jax.Array,
):
    ins = [A_x[0].T, A_wqkv, A_wo, B_u[0].T, B_A_re, B_A_im, B_B_re, B_B_im, B_C_re, B_C_im,
           B_log_dt.reshape(1, D), B_Dskip.reshape(1, D)]
    any_spec = pl.BlockSpec(memory_space=pl.ANY)
    vmem_spec = pl.BlockSpec(memory_space=pltpu.VMEM)
    out = pl.pallas_call(
        _kernel,
        in_specs=[any_spec, any_spec, vmem_spec, any_spec] + [vmem_spec] * 8,
        out_specs=any_spec,
        out_shape=jax.ShapeDtypeStruct((1, S, 2 * D), BF16),
        scratch_shapes=[
            pltpu.VMEM((D, S), BF16),
            pltpu.VMEM((D, 3 * D), BF16),
            pltpu.VMEM((D, S), BF16),
            pltpu.VMEM((S, 2 * D), BF16),
            pltpu.SemaphoreType.DMA((3,)),
            pltpu.SemaphoreType.DMA((NCH,)),
            pltpu.VMEM((4, S, 128), BF16),
            pltpu.VMEM((4, 128, S), BF16),
            pltpu.VMEM((4, S, 128), BF16),
            pltpu.VMEM((4, S, 128), BF16),
            pltpu.VMEM((TQ, S), F32),
            pltpu.VMEM((TQ, S), F32),
            pltpu.VMEM((TQ, S), F32),
            pltpu.VMEM((TQ, S), F32),
            pltpu.VMEM((3 * DP, D), BF16),
            pltpu.VMEM((DP, D), BF16),
            pltpu.VMEM((6, 128, DL), F32),
            pltpu.VMEM((1, DL), F32),
            pltpu.VMEM((40, 128, 128), F32),
            pltpu.VMEM((40, 128, 128), F32),
            pltpu.VMEM((40, 128, 128), F32),
            pltpu.VMEM((40, 128, 128), F32),
            pltpu.VMEM((KROWS, DL), F32),
            pltpu.VMEM((128, DL), F32),
            pltpu.VMEM((NCH, 2 * CH, DPAD), F32),
            pltpu.VMEM((NCH, 2 * CH, DPAD), F32),
            pltpu.VMEM((2 * CH, CH), BF16),
            pltpu.VMEM((2 * CH, 2 * CH), BF16),
            pltpu.VMEM((KROWS, D), BF16),
            pltpu.VMEM((NCH, 2 * CH, DPAD), BF16),
            pltpu.VMEM((CH, D), F32),
            pltpu.VMEM((S, D), F32),
            pltpu.VMEM((2 * CH, 128), BF16),
        ],
        compiler_params=pltpu.CompilerParams(
            vmem_limit_bytes=100 * 1024 * 1024,
        ),
    )(*ins)
    return out
```

```python
import math

import jax
import jax.numpy as jnp
from jax import lax
import jax.experimental.pallas as pl
import jax.experimental.pallas.tpu as pltpu

F32 = jnp.float32
BF16 = jnp.bfloat16

S = 2048
D = 448
H = 16
DH = 28
HP = 32
DP = H * HP
DL = 2 * D
DPAD = 512
NLT = DL // 128
TQ = 512
NQ = S // TQ
NIT = NQ * H
CH = 128
NCH = S // CH
KROWS = 656
UNROLL = 4


def _cmul(ar, ai, br, bi):
    return ar * br - ai * bi, ar * bi + ai * br


def _dot(a, b):
    return jnp.dot(a, b, preferred_element_type=F32)


SR = 32


def _kgen_setup_rows(j, c, prm_ref, dt_ref, xr_ref, xi_ref, yr_ref, yi_ref, k2_ref):
    sl = pl.ds(pl.multiple_of(j * 128, 128), 128)
    rs = pl.ds(pl.multiple_of(c * SR, SR), SR)
    dt = dt_ref[:, sl]
    lr = dt * prm_ref[0, rs, sl]
    li = dt * prm_ref[1, rs, sl]
    dbr = dt * prm_ref[2, rs, sl]
    dbi = dt * prm_ref[3, rs, sl]
    cr, ci = _cmul(prm_ref[4, rs, sl], prm_ref[5, rs, sl], dbr, dbi)
    mag = jnp.exp(lr)
    zr = mag * jnp.cos(li)
    zi = mag * jnp.sin(li)
    pw = [(zr, zi)]
    for _ in range(11):
        r, i = pw[-1]
        pw.append((r * r - i * i, 2.0 * r * i))
    xr, _ = _cmul(cr, ci, pw[11][0], pw[11][1])
    k2_ref[rs, sl] = xr
    yr, yi = jnp.ones_like(zr), jnp.zeros_like(zr)
    for e in range(16):
        yr_ref[e, rs, :] = yr
        yi_ref[e, rs, :] = yi
        if e < 15:
            yr, yi = _cmul(yr, yi, zr, zi)
    for k in range(1, 4):
        yr, yi = pw[k + 3]
        for b in range(8):
            yr_ref[8 + k * 8 + b, rs, :] = yr
            yi_ref[8 + k * 8 + b, rs, :] = yi
            if b < 7:
                yr, yi = _cmul(yr, yi, pw[k][0], pw[k][1])
    blocks = [(None, 0), (7, 0), (8, 1), (9, 2), (10, 3)]
    for blk, (l0, k) in enumerate(blocks):
        if l0 is None:
            xr, xi = (cr, ci)
        else:
            xr, xi = _cmul(cr, ci, pw[l0][0], pw[l0][1])
        sr, si = pw[k + 4]
        for a in range(8):
            xr_ref[blk * 8 + a, rs, :] = xr
            xi_ref[blk * 8 + a, rs, :] = xi
            if a < 7:
                xr, xi = _cmul(xr, xi, sr, si)


def _pow_id(e):
    if e < 16:
        return e
    if e < 32:
        return 8 + (e >> 1)
    if e < 64:
        return 16 + (e >> 2)
    return 24 + (e >> 3)


def _kgen_unit(j, blk, ap, bh, xr_ref, xi_ref, yr_ref, yi_ref, kd_ref):
    off = pl.multiple_of(j * 128, 128)
    xa = blk * 8 + 2 * ap
    yid = [_pow_id((bh * 8 + b) << max(blk - 1, 0)) for b in range(8)]
    acc0 = [None] * 8
    acc1 = [None] * 8
    for r in range(16):
        rs = slice(r * 8, (r + 1) * 8)
        xr0 = xr_ref[xa, rs, :]
        xi0 = xi_ref[xa, rs, :]
        xr1 = xr_ref[xa + 1, rs, :]
        xi1 = xi_ref[xa + 1, rs, :]
        for b in range(8):
            yr = yr_ref[yid[b], rs, :]
            yi = yi_ref[yid[b], rs, :]
            t0 = xr0 * yr - xi0 * yi
            t1 = xr1 * yr - xi1 * yi
            acc0[b] = t0 if acc0[b] is None else acc0[b] + t0
            acc1[b] = t1 if acc1[b] is None else acc1[b] + t1
    b0 = jnp.concatenate([jnp.sum(a, axis=0, keepdims=True) for a in acc0], axis=0)
    b1 = jnp.concatenate([jnp.sum(a, axis=0, keepdims=True) for a in acc1], axis=0)
    r0 = pl.multiple_of(xa * 16 + bh * 8, 8)
    kd_ref[pl.ds(r0, 8), pl.ds(off, 128)] = b0
    kd_ref[pl.ds(r0 + 16, 8), pl.ds(off, 128)] = b1


def _dft_mats():
    f = lax.broadcasted_iota(jnp.int32, (CH, CH), 0)
    t = lax.broadcasted_iota(jnp.int32, (CH, CH), 1)
    ang = (((2 * f + 1) * t) % 512).astype(F32) * (2.0 * math.pi / 512.0)
    fwd = jnp.concatenate([jnp.cos(ang), -jnp.sin(ang)], axis=0)
    t2 = lax.broadcasted_iota(jnp.int32, (2 * CH, CH), 0)
    f2 = lax.broadcasted_iota(jnp.int32, (2 * CH, CH), 1)
    ang2 = (((2 * f2 + 1) * t2) % 512).astype(F32) * (2.0 * math.pi / 512.0)
    inv = jnp.concatenate([jnp.cos(ang2), -jnp.sin(ang2)], axis=1) * (2.0 / 256.0)
    return fwd, inv


def _sel_mat(s, sh, width):
    b = lax.broadcasted_iota(jnp.int32, (CH, width), 0)
    i = lax.broadcasted_iota(jnp.int32, (CH, width), 1)
    q = b >> sh
    rem = b & (s - 1)
    half = s // 2
    up = jnp.logical_or(rem > half, jnp.logical_and(rem == half, (q & 1) == 1))
    q = q + up.astype(jnp.int32)
    return (q == i).astype(BF16)


def _s4_conv(uT_ref, dsk_ref, kd_ref, k2_ref, uf_ref, kf_ref, out_ref, out_hbm, out_sems, fwd_ref, inv_ref, kdb_ref,
             yf_ref, hi_ref, uc_ref, g_ref):
    fwd, inv = _dft_mats()
    fwd_ref[...] = fwd.astype(BF16)
    inv_ref[...] = inv.astype(BF16)
    last = jnp.sum(k2_ref[...], axis=0, keepdims=True)
    row = lax.broadcasted_iota(jnp.int32, (16, DL), 0)
    kd_ref[pl.ds(640, 16), :] = jnp.where(row == 0, last, 0.0)
    kdb_ref[...] = (kd_ref[:, 0:D] + kd_ref[:, D:2 * D]).astype(BF16)
    zpad = jnp.zeros((2 * CH, DPAD - D), F32)

    def fwd_u(a, c):
        r0 = pl.multiple_of(a * CH, CH)
        uc = uT_ref[:, pl.ds(r0, CH)].astype(F32).T
        uc_ref[pl.ds(r0, CH), :] = uc
        uf_ref[a, :, 0:D] = _dot(fwd_ref[...], uc.astype(BF16))
        uf_ref[a, :, D:DPAD] = zpad
        kf_ref[a, :, D:DPAD] = zpad
        return c
    lax.fori_loop(0, NCH, fwd_u, 0)

    def fwd_k0(a, c):
        r0 = pl.multiple_of(a * CH, CH)
        kf_ref[a, :, 0:D] = _dot(fwd_ref[...], kdb_ref[pl.ds(r0, CH), :])
        return c
    lax.fori_loop(0, 2, fwd_k0, 0)

    for (c0, c1, s, sh, base) in ((2, 4, 2, 1, 256), (4, 8, 4, 2, 384), (8, 16, 8, 3, 512)):
        width = CH // s + 16
        g_ref[:, 0:width] = _dot(fwd_ref[...], _sel_mat(s, sh, width)).astype(BF16)

        def fwd_k(a, c, c0=c0, s=s, base=base, width=width):
            r0 = pl.multiple_of(base + (a - c0) * (CH // s), 16)
            kf_ref[a, :, 0:D] = _dot(g_ref[:, 0:width], kdb_ref[pl.ds(r0, width), :])
            return c
        lax.fori_loop(c0, c1, fwd_k, 0)

    RB = 8
    NRB = CH // RB

    def blk_conv(i, c):
        rb = i & (NRB - 1)
        lt = i >> 4
        rr = pl.ds(pl.multiple_of(rb * RB, RB), RB)
        ri = pl.ds(pl.multiple_of(CH + rb * RB, RB), RB)
        ll = pl.ds(pl.multiple_of(lt * 128, 128), 128)
        for a in range(NCH):
            accr = None
            acci = None
            for a2 in range(a + 1):
                ur = uf_ref[a2, rr, ll]
                ui = uf_ref[a2, ri, ll]
                kr = kf_ref[a - a2, rr, ll]
                ki = kf_ref[a - a2, ri, ll]
                pr = ur * kr - ui * ki
                pi = ur * ki + ui * kr
                accr = pr if accr is None else accr + pr
                acci = pi if acci is None else acci + pi
            yf_ref[a, rr, ll] = accr.astype(BF16)
            yf_ref[a, ri, ll] = acci.astype(BF16)
        return c
    lax.fori_loop(0, NRB * (DPAD // 128), blk_conv, 0)

    hi_ref[...] = jnp.zeros(hi_ref.shape, F32)

    def out_chunk(a, c):
        full = _dot(inv_ref[...], yf_ref[a, :, 0:D])
        lo = full[0:CH, :] + hi_ref[...]
        hi_ref[...] = full[CH:2 * CH, :]
        r0 = pl.multiple_of(a * CH, CH)
        uu = uc_ref[pl.ds(r0, CH), :]
        ud = (uu * dsk_ref[...].astype(F32)).astype(BF16).astype(F32)
        out_ref[pl.ds(r0, CH), D:2 * D] = (lo.astype(BF16).astype(F32) + ud).astype(BF16)
        pltpu.make_async_copy(out_ref.at[pl.ds(r0, CH), :], out_hbm.at[0, pl.ds(r0, CH), :],
                              out_sems.at[a]).start()
        return c
    lax.fori_loop(0, NCH, out_chunk, 0)
    for a in range(NCH):
        pltpu.make_async_copy(out_ref.at[pl.ds(a * CH, CH), :],
                              out_hbm.at[0, pl.ds(a * CH, CH), :], out_sems.at[a]).wait()


def _kernel(xT_hbm, wqkv_hbm, wo_ref, uT_hbm, are_ref, aim_ref, bre_ref, bim_ref, cre_ref, cim_ref,
            ldt_ref, dsk_ref,
            out_hbm,
            xT_ref, wqkv_ref, uT_ref, out_ref, in_sems, out_sems,
            q_ref, kT_ref, v_ref, o_ref, sa_ref, sb_ref, sc_ref, sd_ref,
            wpT_ref, wop_ref, prm_ref, dt_ref,
            xr_ref, xi_ref, yr_ref, yi_ref, kd_ref, k2_ref, uf_ref, kf_ref,
            fwd_ref, inv_ref, kdb_ref, yf_ref, hi_ref, uc_ref, g_ref):
    lane = lax.broadcasted_iota(jnp.int32, (TQ, 128), 1)
    lane_head = lane // HP
    qscale = (DH ** -0.5) * math.log2(math.e)

    cp_w = pltpu.make_async_copy(wqkv_hbm, wqkv_ref, in_sems.at[0])
    cp_x = pltpu.make_async_copy(xT_hbm, xT_ref, in_sems.at[1])
    cp_u = pltpu.make_async_copy(uT_hbm, uT_ref, in_sems.at[2])
    cp_w.start()
    cp_x.start()
    cp_u.start()

    for i, p_ref in enumerate((are_ref, aim_ref, bre_ref, bim_ref, cre_ref, cim_ref)):
        pt = p_ref[...].astype(F32).T
        prm_ref[i, :, 0:D] = pt[0:128, :]
        prm_ref[i, :, D:DL] = pt[128:256, :]
    dt = jnp.exp(ldt_ref[...].astype(F32)).astype(BF16).astype(F32)
    dt_ref[:, 0:D] = dt
    dt_ref[:, D:DL] = dt

    def kgen_tile(j, carry):
        def setup(c, cc):
            _kgen_setup_rows(j, c, prm_ref, dt_ref, xr_ref, xi_ref, yr_ref, yi_ref, k2_ref)
            return cc
        lax.fori_loop(0, 128 // SR, setup, 0)

        for blk in range(5):
            for bh in range(2):
                def unit(ap, cc, blk=blk, bh=bh):
                    _kgen_unit(j, blk, ap, bh, xr_ref, xi_ref, yr_ref, yi_ref, kd_ref)
                    return cc
                lax.fori_loop(0, 4, unit, 0)
        return carry
    lax.fori_loop(0, NLT, kgen_tile, 0)

    cp_w.wait()
    cp_x.wait()

    wT = wqkv_ref[...].astype(F32).T.astype(BF16)
    zrows = jnp.zeros((HP - DH, D), BF16)
    for g in range(3 * H):
        wpT_ref[g * HP:g * HP + DH, :] = wT[g * DH:(g + 1) * DH, :]
        wpT_ref[g * HP + DH:(g + 1) * HP, :] = zrows
    for g in range(H):
        wop_ref[g * HP:g * HP + DH, :] = wo_ref[g * DH:(g + 1) * DH, :]
        wop_ref[g * HP + DH:(g + 1) * HP, :] = zrows

    def proj(i, c):
        r0 = pl.multiple_of(i * TQ, TQ)
        xb = xT_ref[:, pl.ds(r0, TQ)]
        qkvT = _dot(wpT_ref[...], xb)
        q = (qkvT[0:DP, :] * qscale).T.astype(BF16)
        kt = qkvT[DP:2 * DP, :].astype(BF16)
        rowh = lax.broadcasted_iota(jnp.int32, (DP, TQ), 0)
        v = jnp.where(rowh % HP == DH, 1.0, qkvT[2 * DP:3 * DP, :]).T.astype(BF16)
        for t in range(4):
            q_ref[t, pl.ds(r0, TQ), :] = q[:, t * 128:(t + 1) * 128]
            v_ref[t, pl.ds(r0, TQ), :] = v[:, t * 128:(t + 1) * 128]
            kT_ref[t, :, pl.ds(r0, TQ)] = kt[t * 128:(t + 1) * 128, :]
            o_ref[t, pl.ds(r0, TQ), :] = jnp.zeros((TQ, 128), BF16)
        return c
    lax.fori_loop(0, NQ, proj, 0)

    def scores(it):
        qb = it >> 4
        h = it & 15
        t = h >> 2
        r0 = pl.multiple_of(qb * TQ, TQ)
        qt = q_ref[t, pl.ds(r0, TQ), :]
        qm = jnp.where(lane_head == (h & 3), qt, jnp.zeros_like(qt))
        return _dot(qm, kT_ref[t])

    def softmax_pv(it, s_in_ref):
        qb = it >> 4
        h = it & 15
        t = h >> 2
        hh = h & 3
        r0 = pl.multiple_of(qb * TQ, TQ)
        s = s_in_ref[...]
        m = jnp.max(s, axis=-1, keepdims=True)
        p = jnp.exp2(s - m).astype(BF16)
        o = _dot(p, v_ref[t])
        l = jnp.sum(jnp.where(lane == hh * HP + DH, o, 0.0), axis=-1, keepdims=True)
        on = (o / l).astype(BF16)
        o_ref[t, pl.ds(r0, TQ), :] = jnp.where(lane_head == hh, on, o_ref[t, pl.ds(r0, TQ), :])

    sbufs = (sa_ref, sb_ref, sc_ref, sd_ref)
    sa_ref[...] = scores(0)
    sb_ref[...] = scores(1)

    def main(i4, c):
        it0 = i4 * UNROLL
        for k4 in range(UNROLL):
            it = it0 + k4
            sbufs[(k4 + 2) % 4][...] = scores(it + 2)
            softmax_pv(it, sbufs[k4 % 4])
        return c
    lax.fori_loop(0, NIT // UNROLL - 1, main, 0)
    for k4 in range(UNROLL):
        it = NIT - UNROLL + k4
        if it + 2 < NIT:
            sbufs[(k4 + 2) % 4][...] = scores(it + 2)
        softmax_pv(it, sbufs[k4 % 4])

    def oproj(i, c):
        r0 = pl.multiple_of(i * TQ, TQ)
        oall = jnp.concatenate([o_ref[t, pl.ds(r0, TQ), :] for t in range(4)], axis=1)
        out_ref[pl.ds(r0, TQ), 0:D] = _dot(oall, wop_ref[...]).astype(BF16)
        return c
    lax.fori_loop(0, NQ, oproj, 0)

    cp_u.wait()
    _s4_conv(uT_ref, dsk_ref, kd_ref, k2_ref, uf_ref, kf_ref, out_ref, out_hbm, out_sems,
             fwd_ref, inv_ref, kdb_ref, yf_ref, hi_ref, uc_ref, g_ref)


@jax.jit
def pallas_concat_heads__mha_block__ssm_conv_s4__prompt_kernel(
    A_x: jax.Array,
    A_wqkv: jax.Array,
    A_wo: jax.Array,
    B_u: jax.Array,
    B_A_re: jax.Array,
    B_A_im: jax.Array,
    B_B_re: jax.Array,
    B_B_im: jax.Array,
    B_C_re: jax.Array,
    B_C_im: jax.Array,
    B_log_dt: jax.Array,
    B_Dskip: jax.Array,
):
    ins = [A_x[0].T, A_wqkv, A_wo, B_u[0].T, B_A_re, B_A_im, B_B_re, B_B_im, B_C_re, B_C_im,
           B_log_dt.reshape(1, D), B_Dskip.reshape(1, D)]
    any_spec = pl.BlockSpec(memory_space=pl.ANY)
    vmem_spec = pl.BlockSpec(memory_space=pltpu.VMEM)
    out = pl.pallas_call(
        _kernel,
        in_specs=[any_spec, any_spec, vmem_spec, any_spec] + [vmem_spec] * 8,
        out_specs=any_spec,
        out_shape=jax.ShapeDtypeStruct((1, S, 2 * D), BF16),
        scratch_shapes=[
            pltpu.VMEM((D, S), BF16),
            pltpu.VMEM((D, 3 * D), BF16),
            pltpu.VMEM((D, S), BF16),
            pltpu.VMEM((S, 2 * D), BF16),
            pltpu.SemaphoreType.DMA((3,)),
            pltpu.SemaphoreType.DMA((NCH,)),
            pltpu.VMEM((4, S, 128), BF16),
            pltpu.VMEM((4, 128, S), BF16),
            pltpu.VMEM((4, S, 128), BF16),
            pltpu.VMEM((4, S, 128), BF16),
            pltpu.VMEM((TQ, S), F32),
            pltpu.VMEM((TQ, S), F32),
            pltpu.VMEM((TQ, S), F32),
            pltpu.VMEM((TQ, S), F32),
            pltpu.VMEM((3 * DP, D), BF16),
            pltpu.VMEM((DP, D), BF16),
            pltpu.VMEM((6, 128, DL), F32),
            pltpu.VMEM((1, DL), F32),
            pltpu.VMEM((40, 128, 128), F32),
            pltpu.VMEM((40, 128, 128), F32),
            pltpu.VMEM((40, 128, 128), F32),
            pltpu.VMEM((40, 128, 128), F32),
            pltpu.VMEM((KROWS, DL), F32),
            pltpu.VMEM((128, DL), F32),
            pltpu.VMEM((NCH, 2 * CH, DPAD), F32),
            pltpu.VMEM((NCH, 2 * CH, DPAD), F32),
            pltpu.VMEM((2 * CH, CH), BF16),
            pltpu.VMEM((2 * CH, 2 * CH), BF16),
            pltpu.VMEM((KROWS, D), BF16),
            pltpu.VMEM((NCH, 2 * CH, DPAD), BF16),
            pltpu.VMEM((CH, D), F32),
            pltpu.VMEM((S, D), F32),
            pltpu.VMEM((2 * CH, 128), BF16),
        ],
        compiler_params=pltpu.CompilerParams(
            vmem_limit_bytes=100 * 1024 * 1024,
        ),
    )(*ins)
    return out
```
